```python
import os as _os
_os.environ.setdefault("JAX_PLATFORMS", "cpu")
import jax
import jax.numpy as jnp

def _softmax(x, axis=-1):
    return jax.nn.softmax(x, axis=axis)
def _gelu(x):
    return jax.nn.gelu(x, approximate=True)
def _silu(x):
    return jax.nn.silu(x)
def _sigmoid(x):
    return jax.nn.sigmoid(x)
def _layernorm(x, axis=-1, eps=1e-5):
    m = jnp.mean(x, axis=axis, keepdims=True)
    v = jnp.var(x, axis=axis, keepdims=True)
    return (x - m) / jnp.sqrt(v + eps)
def _scatter_add(tgt, idx, src, axis=0):
    return tgt.at[idx].add(src)
def _segment_sum(src, seg, n):
    return jax.ops.segment_sum(src, seg, n)
class _Rng:
    def __init__(self, key):
        self._k = key
    def _next(self):
        self._k, sub = jax.random.split(self._k)
        return sub
    def normal(self, shape):
        return jax.random.normal(self._next(), shape, dtype=jnp.bfloat16)
    def randint(self, lo, hi, shape):
        return jax.random.randint(self._next(), shape, lo, hi, dtype=jnp.int32)
    def uniform(self, shape, lo=0.0, hi=1.0):
        return jax.random.uniform(self._next(), shape, jnp.bfloat16, lo, hi)
    def permutation(self, n):
        return jax.random.permutation(self._next(), n)


kernel_name = 'concat_heads__gqa_block_cached__mha_block_cached__near_ridge'

def setup_inputs():
    _rng = _Rng(jax.random.key(int.from_bytes(__import__("os").urandom(4), "little")))
    _w = (lambda a: (lambda t: t.astype(jnp.bfloat16) if jnp.issubdtype(t.dtype, jnp.floating) else t)(jnp.asarray(a)))
    def _A_setup():
        B, Sq, D = 8, 96, 640
        Hq, Hkv, Sk, Dh = 32, 32, 512, 128
        assert Hq % Hkv == 0, (Hq, Hkv)
        return {
            "x": _w((lambda *s: _rng.normal(s) * 0.8)(B, Sq, D)),
            "k_cache": _w((lambda *s: _rng.normal(s) * 0.8)(B, Hkv, Sk, Dh)),
            "v_cache": _w((lambda *s: _rng.normal(s) * 0.05)(B, Hkv, Sk, Dh)),
            "wq": _w((lambda *s: _rng.normal(s) * 0.8)(D, Hq * Dh) * (D ** -0.5)),
            "wo": _w((lambda *s: _rng.normal(s) * 0.05)(Hq * Dh, D) * ((Hq * Dh) ** -0.5)),
        }
    _A_in = _A_setup()

    def _B_setup():
        B, Sq, D = 8, 96, 640
        H, Sk, Dh = 32, 512, 128
        return {
            "x": _w((lambda *s: _rng.normal(s) * 0.8)(B, Sq, D)),
            "k_cache": _w((lambda *s: _rng.normal(s) * 0.8)(B, H, Sk, Dh)),
            "v_cache": _w((lambda *s: _rng.normal(s) * 0.05)(B, H, Sk, Dh)),
            "wq": _w((lambda *s: _rng.normal(s) * 0.8)(D, H * Dh) * (D ** -0.5)),
            "wo": _w((lambda *s: _rng.normal(s) * 0.05)(H * Dh, D) * ((H * Dh) ** -0.5)),
        }
    _B_in = _B_setup()

    return {
        "A_x": _A_in["x"],
        "A_k_cache": _A_in["k_cache"],
        "A_v_cache": _A_in["v_cache"],
        "A_wq": _A_in["wq"],
        "A_wo": _A_in["wo"],
        "B_x": _B_in["x"],
        "B_k_cache": _B_in["k_cache"],
        "B_v_cache": _B_in["v_cache"],
        "B_wq": _B_in["wq"],
        "B_wo": _B_in["wo"],
    }

def reference(A_x, A_k_cache, A_v_cache, A_wq, A_wo, B_x, B_k_cache, B_v_cache, B_wq, B_wo):
    def _A_ref(x, k_cache, v_cache, wq, wo):
        B, Sq, D = x.shape
        Hq, Dh = 32, 128
        Hkv = k_cache.shape[1]
        rep = Hq // Hkv
        q = (lambda x, *d: x.transpose(*d))((x @ wq).reshape(B, Sq, Hq, Dh), 0, 2, 1, 3)
        k = jnp.repeat(k_cache, rep, axis=1)
        v = jnp.repeat(v_cache, rep, axis=1)
        scores = jnp.einsum("bhqd,bhkd->bhqk", q, k) * (Dh ** -0.5)
        p = _softmax(scores, axis=-1)
        o = jnp.einsum("bhqk,bhkd->bhqd", p, v)
        return (lambda x, *d: x.transpose(*d))(o, 0, 2, 1, 3).reshape(B, Sq, Hq * Dh) @ wo

    def _B_ref(x, k_cache, v_cache, wq, wo):
        B, Sq, D = x.shape
        H, Dh = 32, 128
        q = (lambda x, *d: x.transpose(*d))((x @ wq).reshape(B, Sq, H, Dh), 0, 2, 1, 3)
        scores = jnp.einsum("bhqd,bhkd->bhqk", q, k_cache) * (Dh ** -0.5)
        p = _softmax(scores, axis=-1)
        o = jnp.einsum("bhqk,bhkd->bhqd", p, v_cache)
        return (lambda x, *d: x.transpose(*d))(o, 0, 2, 1, 3).reshape(B, Sq, H * Dh) @ wo

    a = _A_ref(A_x, A_k_cache, A_v_cache, A_wq, A_wo)
    b = _B_ref(B_x, B_k_cache, B_v_cache, B_wq, B_wo)
    return jnp.concatenate([a, b], axis=-1)
```

```python
import math
import jax, jax.numpy as jnp
from jax import lax
from jax.experimental import pallas as pl
from jax.experimental.pallas import tpu as pltpu

B,SQ,D,H,SK,DH = 8,96,640,32,512,128
HG = 4; W = HG*DH; NG = H//HG; UB = NG*B; U = 2*UB
QS = (DH**-0.5)*math.log2(math.e)
NT = (((1,),(1,)),((),()))
f32 = jnp.float32; bf = jnp.bfloat16

def make(order="k0 k1 k2 k3 o v0 v1 v2 v3 q", ns=4, dma=True, flags=None, unroll=1, prio=(0,0,0,0), nw=3):
    order = order.split()
    def kern(ax,ak,av,awq,awo,bx,bk,bv,bwq,bwo,out,kb,vb,wqb,wob,xb,qb,ob,acc,outb,ksem,vsem,wsem,xsem,osem):
        hb = ((ax,ak,av,awq,awo),(bx,bk,bv,bwq,bwo))
        def kv_copies(br, g, b, slot):
            return [pltpu.make_async_copy(hb[br][1].at[b,pl.ds(g*HG,HG)], kb.at[slot], ksem.at[slot]),
                    pltpu.make_async_copy(hb[br][2].at[b,pl.ds(g*HG,HG)], vb.at[slot], vsem.at[slot])]
        def wq_copy(br, g, slot):
            return pltpu.make_async_copy(hb[br][3].at[:,pl.ds(pl.multiple_of(g*W,W),W)], wqb.at[slot], wsem.at[0,slot])
        def wo_copy(br, g, slot):
            return pltpu.make_async_copy(hb[br][4].at[pl.ds(pl.multiple_of(g*W,W),W)], wob.at[slot], wsem.at[1,slot])
        def x_copy(br): return pltpu.make_async_copy(hb[br][0], xb.at[br], xsem.at[br])
        def o_copy(br, b): return pltpu.make_async_copy(outb.at[br,b], out.at[b,:,pl.ds(br*D,D)], osem.at[br,b])
        def start_unit(u):
            for br in range(2):
                def go(br=br):
                    r = u-br*UB; g = r//B; b = r%B; gg = u//B
                    def wq_(): wq_copy(br,g,gg%nw).start(priority=prio[2])
                    def wo_(): wo_copy(br,g,gg%nw).start(priority=prio[3])
                    if isinstance(u,int):
                        if b==0: wq_()
                    else: pl.when(b==0)(wq_)
                    for j,c in enumerate(kv_copies(br,g,b,u%ns)): c.start(priority=prio[j])
                    if isinstance(u,int):
                        if b==0: wo_()
                    else: pl.when(b==0)(wo_)
                if isinstance(u,int):
                    if u//UB==br: go()
                else: pl.when(u//UB==br)(go)
        def qproj(u):
            q = jnp.dot(xb[u//UB, u%B], wqb[(u//B)%nw], preferred_element_type=f32)*QS
            qb[u%2] = q.astype(bf)
        def oproj(u):
            br = u//UB; b = u%B
            r = acc[br,b] + jnp.dot(ob[u%2], wob[(u//B)%nw], preferred_element_type=f32)
            acc[br,b] = r
            outb[br,b] = r.astype(bf)
        def step(u, first=False, last=False):
            slot = u%ns
            if dma:
                if not last:
                    @pl.when((u+1)%B==0)
                    def _(): wq_copy(0,0,((u+1)//B)%nw).wait()
                    @pl.when(u+1==UB)
                    def _(): x_copy(1).wait()
                if not first:
                    @pl.when((u-1)%B==0)
                    def _(): wo_copy(0,0,((u-1)//B)%nw).wait()
                for c in kv_copies(0,0,0,slot): c.wait()
            st = {}
            for op in order:
                if op=="q":
                    if not last: qproj(u+1)
                elif op=="o":
                    if not first: oproj(u-1)
                elif op[0]=="k":
                    h = int(op[1])
                    s = lax.dot_general(qb[u%2,:,h*DH:(h+1)*DH], kb[slot,h], NT, preferred_element_type=f32)
                    m = jnp.max(s,axis=1,keepdims=True)
                    p = jnp.exp2(s-m)
                    st[h] = (p.astype(bf), 1.0/jnp.sum(p,axis=1,keepdims=True))
                else:
                    h = int(op[1]); p, r = st[h]
                    o = jnp.dot(p, vb[slot,h], preferred_element_type=f32)
                    ob[u%2,:,h*DH:(h+1)*DH] = (o*r).astype(bf)
            if dma and not last:
                if isinstance(u,int): start_unit(u+ns)
                else: pl.when(u+ns<U)(lambda: start_unit(u+ns))
            if not first:
                for br in range(2):
                    @pl.when((u-1)//B==br*NG+NG-1)
                    def _(): o_copy(br,(u-1)%B).start()
        x_copy(0).start()
        for u in range(ns): start_unit(u)
        x_copy(1).start()
        acc[...] = jnp.zeros_like(acc)
        x_copy(0).wait(); wq_copy(0,0,0).wait()
        if not dma:
            x_copy(1).wait()
            for u in range(ns):
                for c in kv_copies(0,0,0,u): c.wait()
                if u%B==0:
                    wo_copy(0,0,u//B).wait()
                    if u: wq_copy(0,0,u//B).wait()
        qproj(0)
        step(0, first=True)
        def body(i,_):
            for j in range(unroll): step(1+i*unroll+j)
        lax.fori_loop(0,(U-2)//unroll,body,None)
        step(U-1, last=True)
        oproj(U-1)
        o_copy(1,B-1).start()
        for br in range(2):
            for b in range(B): o_copy(br,b).wait()
    f = pl.pallas_call(kern, out_shape=jax.ShapeDtypeStruct((B,SQ,2*D),bf),
        in_specs=[pl.BlockSpec(memory_space=pl.ANY)]*10, out_specs=pl.BlockSpec(memory_space=pl.ANY),
        scratch_shapes=[pltpu.VMEM((ns,HG,SK,DH),bf),pltpu.VMEM((ns,HG,SK,DH),bf),
            pltpu.VMEM((nw,D,W),bf),pltpu.VMEM((nw,W,D),bf),pltpu.VMEM((2,B,SQ,D),bf),
            pltpu.VMEM((2,SQ,W),bf),pltpu.VMEM((2,SQ,W),bf),pltpu.VMEM((2,B,SQ,D),f32),pltpu.VMEM((2,B,SQ,D),bf),
            pltpu.SemaphoreType.DMA((ns,)),pltpu.SemaphoreType.DMA((ns,)),pltpu.SemaphoreType.DMA((2,nw)),
            pltpu.SemaphoreType.DMA((2,)),pltpu.SemaphoreType.DMA((2,B))],
        compiler_params=pltpu.CompilerParams(vmem_limit_bytes=100*2**20, flags=flags))
    return f


@jax.jit
def pallas_concat_heads__gqa_block_cached__mha_block_cached__near_ridge_kernel(
    A_x, A_k_cache, A_v_cache, A_wq, A_wo, B_x, B_k_cache, B_v_cache, B_wq, B_wo):
    return make()(A_x, A_k_cache, A_v_cache, A_wq, A_wo, B_x, B_k_cache, B_v_cache, B_wq, B_wo)
```

```python
import math

import jax
import jax.numpy as jnp
from jax import lax
from jax.experimental import pallas as pl
from jax.experimental.pallas import tpu as pltpu

B, SQ, D = 8, 96, 640
H, SK, DH = 32, 512, 128

G = 4
GW = G * DH
BRANCH_STEPS = (H // G) * B
STEPS = 2 * BRANCH_STEPS

KV_SLOTS = 4
W_SLOTS = 4
Q_SLOTS = 4
KV_AHEAD = 3
Q_AHEAD = 6
WQ_AHEAD = Q_AHEAD + B - 1
WO_AHEAD = 5
X_B_GROUP = 4
FIRST_Q = 4

KV_ROWS = 128
WQ_ROWS = (24, 24, 16, 16)
WO_ROWS = (16, 16, 16, 16)
X_ROWS = 24
OUT_ROWS = 48

Q_SCALE = DH ** -0.5 * math.log2(math.e)
NT_DIMS = (((1,), (1,)), ((), ()))
F32, BF16 = jnp.float32, jnp.bfloat16


def _div(a, c):
    if isinstance(a, int):
        return a // c
    return lax.shift_right_logical(a, c.bit_length() - 1)


def _mod(a, c):
    return a & (c - 1)


def _rows(start, size, align):
    return pl.ds(start if isinstance(start, int) else pl.multiple_of(start, align), size)


def _loop(lo, hi, body):
    lax.fori_loop(lo, hi, lambda n, _: body(n), None)


def _start(copies):
    for j, copy in enumerate(copies):
        copy.start(priority=j % 2)


def _wait_all(buf, sem):
    pltpu.make_async_copy(buf, buf, sem).wait()


def _batch(n, i):
    return _mod(_div(n, G), 2) + 2 * i


def _kernel(ax, ak, av, awq, awo, bx, bk, bv, bwq, bwo, out,
            kv_buf, wq_buf, wo_buf, x_buf, q_buf, o_buf, acc, out_buf, sems):
    x_hbm, kv_hbm = (ax, bx), ((ak, av), (bk, bv))
    wq_hbm, wo_hbm = (awq, bwq), (awo, bwo)

    kv_sem = lambda a, slot: sems.at[a * KV_SLOTS + slot]
    wq_sem = lambda slot: sems.at[2 * KV_SLOTS + slot]
    wo_sem = lambda slot: sems.at[2 * KV_SLOTS + W_SLOTS + slot]
    x_sem = lambda br: sems.at[2 * KV_SLOTS + 2 * W_SLOTS + br]
    out_sem = lambda br: sems.at[2 * KV_SLOTS + 2 * W_SLOTS + 2 + br]
    w_slot = lambda n: _mod(_div(n, B), W_SLOTS)

    def kv_copies(br, n, chunk, by_batch=False):
        r, slot = n - br * BRANCH_STEPS, _mod(n, KV_SLOTS)
        rows = _rows(chunk * KV_ROWS, KV_ROWS, KV_ROWS)
        copies = []
        for a in range(2):
            for i in range(G):
                bi, hi = (_mod(r, G), i) if by_batch else (i, _mod(r, G))
                copies.append(pltpu.make_async_copy(
                    kv_hbm[br][a].at[_batch(r, bi), _div(r, B) * G + hi, rows],
                    kv_buf.at[slot, a, i, rows], kv_sem(a, slot)))
        return copies

    def wq_copies(br, n):
        r, first, copies = n - br * BRANCH_STEPS, 0, []
        for size in WQ_ROWS:
            rows = _rows(_mod(r, B) * (D // B) + first, size, 8)
            copies.append(pltpu.make_async_copy(
                wq_hbm[br].at[rows, _rows(_div(r, B) * GW, GW, GW)],
                wq_buf.at[w_slot(n), rows], wq_sem(w_slot(n))))
            first += size
        return copies

    def wo_copies(br, n):
        r, first, copies = n - br * BRANCH_STEPS, 0, []
        for size in WO_ROWS:
            copies.append(pltpu.make_async_copy(
                wo_hbm[br].at[_rows(r * (GW // B) + first, size, 8)],
                wo_buf.at[w_slot(n), _rows(_mod(r, B) * (GW // B) + first, size, 8)],
                wo_sem(w_slot(n))))
            first += size
        return copies

    def x_copies(br, j):
        return [pltpu.make_async_copy(
            x_hbm[br].at[_batch(j, _mod(j, G)), pl.ds(i, X_ROWS)],
            x_buf.at[br, j, pl.ds(i, X_ROWS)], x_sem(br)) for i in range(0, SQ, X_ROWS)]

    def out_copy(br, j, first, size):
        return pltpu.make_async_copy(
            out_buf.at[br, j, pl.ds(first, size)],
            out.at[_batch(j, _mod(j, G)), pl.ds(first, size), pl.ds(br * D, D)], out_sem(br))

    def start_unit(m, kv_br, wq_br=None, wo_br=None, by_batch=False):
        wq = [] if wq_br is None else wq_copies(wq_br, m + WQ_AHEAD)
        wo = [] if wo_br is None else wo_copies(wo_br, m + WO_AHEAD)
        extra = (wq[:2], wo[:2], wq[2:], wo[2:])
        _start([c for chunk in range(SK // KV_ROWS)
                for c in extra[chunk] + kv_copies(kv_br, m, chunk, by_batch)])

    def start_any_unit(m, cases):
        if len(cases) == 1:
            return start_unit(m, *cases[0][1])
        half = len(cases) // 2
        lax.cond(m < cases[half][0],
                 lambda: start_any_unit(m, cases[:half]),
                 lambda: start_any_unit(m, cases[half:]))

    def q_proj(n):
        q = jnp.dot(x_buf[_div(n, BRANCH_STEPS), _mod(n, B)], wq_buf[w_slot(n)],
                    preferred_element_type=F32)
        q = (q * Q_SCALE).astype(BF16)
        for h in range(G):
            q_buf[_mod(_div(n, G), Q_SLOTS), _mod(n, G), h] = q[:, h * DH:(h + 1) * DH]

    def out_proj(n):
        o = jnp.concatenate(
            [o_buf[_mod(_div(n, G), 2), _mod(n, G), h] for h in range(G)], axis=1)
        total = jnp.where(_mod(n, BRANCH_STEPS) >= B, acc[_mod(n, B)], 0.0)
        total += jnp.dot(o, wo_buf[w_slot(n)], preferred_element_type=F32)
        acc[_mod(n, B)] = total
        out_buf[_mod(_div(n, BRANCH_STEPS), 2), _mod(n, B)] = total.astype(BF16)

    def probs(n, i, pos):
        s = lax.dot_general(q_buf[(_mod(_div(n, G), Q_SLOTS),) + pos],
                            kv_buf[_mod(n, KV_SLOTS), 0, i], NT_DIMS,
                            preferred_element_type=F32)
        p = jnp.exp2(s - jnp.max(s, axis=1, keepdims=True))
        return p.astype(BF16), 1.0 / jnp.sum(p, axis=1, keepdims=True)

    def values(n, i, pos, p, inv_sum):
        o = jnp.dot(p, kv_buf[_mod(n, KV_SLOTS), 1, i], preferred_element_type=F32)
        o_buf[(_mod(_div(n, G), 2),) + pos] = (o * inv_sum).astype(BF16)

    def wait_kv(n):
        for a in range(2):
            _wait_all(kv_buf.at[_mod(n, KV_SLOTS), a], kv_sem(a, _mod(n, KV_SLOTS)))

    def wait_wo(n):
        _wait_all(wo_buf.at[w_slot(n)], wo_sem(w_slot(n)))

    _loop(0, G, lambda j: _start(
        x_copies(0, j) + x_copies(0, j + G) + wq_copies(0, j) + wq_copies(0, j + G)))

    def clear(j):
        acc[j] = jnp.zeros((SQ, D), F32)
        for h in range(2):
            o_buf[1, _div(j, 2), 2 * _mod(j, 2) + h] = jnp.zeros((SQ, DH), BF16)
        wo_buf[W_SLOTS - 1, _rows(j * (GW // B), GW // B, GW // B)] = (
            jnp.zeros((GW // B, D), BF16))

    _loop(0, B, clear)

    def prologue(j):
        chunks = SK // KV_ROWS

        @pl.when(j < B)
        def _():
            kv = kv_copies(0, _div(j, chunks), _mod(j, chunks))
            wq, wo = wq_copies(0, B + j), wo_copies(0, j)
            _start(wq[:2] + kv[:2] + wo[:2] + kv[2:4] + wq[2:] + kv[4:6] + wo[2:] + kv[6:])

        @pl.when(j >= B)
        def _():
            _start(kv_copies(0, _div(j, chunks), _mod(j, chunks)))

        @pl.when(j == FIRST_Q)
        def _():
            _wait_all(x_buf.at[0], x_sem(0))
            _wait_all(wq_buf.at[0], wq_sem(0))

        pl.when((j >= FIRST_Q) & (j < FIRST_Q + Q_AHEAD))(lambda: q_proj(j - FIRST_Q))

    _loop(0, KV_AHEAD * (SK // KV_ROWS), prologue)

    def step(n):
        nq = n + Q_AHEAD
        pl.when(_mod(n, B) == G)(lambda: wait_wo(n))
        pl.when(_mod(nq, B) == 0)(
            lambda: _wait_all(wq_buf.at[w_slot(nq)], wq_sem(w_slot(nq))))
        pl.when(nq == BRANCH_STEPS)(lambda: _wait_all(x_buf.at[1], x_sem(1)))
        wait_kv(n)
        start_any_unit(n + KV_AHEAD, [
            (0, (0, 0, 0)),
            (BRANCH_STEPS - WQ_AHEAD, (0, 1, 0)),
            (BRANCH_STEPS - WO_AHEAD, (0, 1, 1)),
            (BRANCH_STEPS, (1, 1, 1)),
            (STEPS - WQ_AHEAD, (1, None, 1)),
            (STEPS - WO_AHEAD, (1,)),
            (STEPS - G, (1, None, None, True)),
        ])
        pl.when(_div(n, B) == X_B_GROUP)(lambda: _start(x_copies(1, _mod(n, B))))
        out_proj(n - G + STEPS)
        p = [probs(n, i, (i, _mod(n, G))) for i in range(G)]
        q_proj(nq)
        for i in range(G):
            values(n, i, (i, _mod(n, G)), *p[i])

    _loop(0, STEPS - Q_AHEAD, step)

    def late_step(n):
        wait_kv(n)
        p = [probs(n, i, (i, _mod(n, G))) for i in range(G)]
        out_proj(n - G)
        for i in range(G):
            values(n, i, (i, _mod(n, G)), *p[i])
        start_unit(n + KV_AHEAD, 1, by_batch=True)

    _loop(STEPS - Q_AHEAD, STEPS - G, late_step)

    wait_wo(STEPS - G)

    def last_step(n):
        j = _mod(n, G)
        wait_kv(n)
        pl.when(j == 1)(lambda: start_unit(STEPS - 1, 1, by_batch=True))
        pl.when(j == 2)(lambda: _start(
            [out_copy(0, i, 0, SQ) for i in range(B)] + [out_copy(1, i, 0, SQ) for i in range(G)]))
        p = [probs(n, i, (j, i)) for i in range(2)]
        out_proj(STEPS - B + 2 * j)
        p += [probs(n, i, (j, i)) for i in range(2, G)]
        for i in range(G):
            values(n, i, (j, i), *p[i])
        out_proj(STEPS - B + 2 * j + 1)
        pl.when(j >= 2)(lambda: _start(
            [out_copy(1, 2 * j + i, first, OUT_ROWS)
             for first in range(0, SQ, OUT_ROWS) for i in range(2)]))

    _loop(STEPS - G, STEPS, last_step)

    for br in range(2):
        _wait_all(out_buf.at[br], out_sem(br))


@jax.jit
def pallas_concat_heads__gqa_block_cached__mha_block_cached__near_ridge_kernel(
    A_x: jax.Array,
    A_k_cache: jax.Array,
    A_v_cache: jax.Array,
    A_wq: jax.Array,
    A_wo: jax.Array,
    B_x: jax.Array,
    B_k_cache: jax.Array,
    B_v_cache: jax.Array,
    B_wq: jax.Array,
    B_wo: jax.Array,
):
    args = (A_x, A_k_cache, A_v_cache, A_wq, A_wo, B_x, B_k_cache, B_v_cache, B_wq, B_wo)
    shapes = ((B, SQ, D), (B, H, SK, DH), (B, H, SK, DH), (D, H * DH), (H * DH, D))
    assert tuple(a.shape for a in args) == 2 * shapes
    assert WQ_AHEAD + KV_AHEAD == 2 * B and WO_AHEAD + KV_AHEAD == B

    return pl.pallas_call(
        _kernel,
        out_shape=jax.ShapeDtypeStruct((B, SQ, 2 * D), BF16),
        in_specs=[pl.BlockSpec(memory_space=pl.ANY)] * len(args),
        out_specs=pl.BlockSpec(memory_space=pl.ANY),
        scratch_shapes=[
            pltpu.VMEM((KV_SLOTS, 2, G, SK, DH), BF16),
            pltpu.VMEM((W_SLOTS, D, GW), BF16),
            pltpu.VMEM((W_SLOTS, GW, D), BF16),
            pltpu.VMEM((2, B, SQ, D), BF16),
            pltpu.VMEM((Q_SLOTS, G, G, SQ, DH), BF16),
            pltpu.VMEM((2, G, G, SQ, DH), BF16),
            pltpu.VMEM((B, SQ, D), F32),
            pltpu.VMEM((2, B, SQ, D), BF16),
            pltpu.SemaphoreType.DMA((2 * KV_SLOTS + 2 * W_SLOTS + 4,)),
        ],
        compiler_params=pltpu.CompilerParams(
            vmem_limit_bytes=64 * 2**20, disable_bounds_checks=True),
    )(*(a.astype(BF16) for a in args))
```

```python
import math

import jax
import jax.numpy as jnp
from jax import lax
from jax.experimental import pallas as pl
from jax.experimental.pallas import tpu as pltpu

B, SQ, D = 8, 96, 640
H, SK, DH = 32, 512, 128

G = 4
GW = G * DH
HW = H * DH // 2
BRANCH_STEPS = (H // G) * B
STEPS = 2 * BRANCH_STEPS

KV_SLOTS = 4
WO_SLOTS = 4
Q_SLOTS = 4
KV_AHEAD = 3
WO_AHEAD = B - KV_AHEAD
Q_AHEAD = 5

KV_ROWS = 128
CHUNKS = SK // KV_ROWS
WQ_ROWS = 8
WO_TILES = 16
GROUP_TILES = (GW // 8) * (D // DH)
X_ROWS = 24
OUT_ROWS = 48

Q_SCALE = DH ** -0.5 * math.log2(math.e)
NT_DIMS = (((1,), (1,)), ((), ()))
F32, BF16 = jnp.float32, jnp.bfloat16


def _div(a, c):
    if isinstance(a, int):
        return a // c
    return lax.shift_right_logical(a, c.bit_length() - 1)


def _mod(a, c):
    return a & (c - 1)


def _rows(start, size, align):
    return pl.ds(start if isinstance(start, int) else pl.multiple_of(start, align), size)


def _loop(lo, hi, body):
    lax.fori_loop(lo, hi, lambda n, _: body(n), None)


def _start(copies):
    for j, copy in enumerate(copies):
        copy.start(priority=j % 2)


def _wait_all(buf, sem):
    pltpu.make_async_copy(buf, buf, sem).wait()


def _batch(n, i):
    return _mod(_div(n, G), 2) + 2 * i


def _kernel(ax, ak, av, awq, awo, bx, bk, bv, bwq, bwo, out,
            kv_buf, wq_buf, wo_buf, x_buf, q_buf, o_buf, acc, out_buf, sems):
    x_hbm, kv_hbm = (ax, bx), ((ak, av), (bk, bv))
    wq_hbm, wo_hbm = (awq, bwq), (awo, bwo)

    kv_sem = lambda a, slot: sems.at[a * KV_SLOTS + slot]
    wo_sem = lambda slot: sems.at[2 * KV_SLOTS + slot]
    wq_sem = lambda half: sems.at[2 * KV_SLOTS + WO_SLOTS + half]
    x_sem = lambda br: sems.at[2 * KV_SLOTS + WO_SLOTS + 4 + br]
    out_sem = sems.at[2 * KV_SLOTS + WO_SLOTS + 6]
    wo_slot = lambda n: _mod(_div(n, B), WO_SLOTS)

    def kv_copies(br, n, chunk, by_batch=False):
        r, slot = n - br * BRANCH_STEPS, _mod(n, KV_SLOTS)
        rows = _rows(chunk * KV_ROWS, KV_ROWS, KV_ROWS)
        copies = []
        for a in range(2):
            for i in range(G):
                bi, hi = (_mod(r, G), i) if by_batch else (i, _mod(r, G))
                copies.append(pltpu.make_async_copy(
                    kv_hbm[br][a].at[_batch(r, bi), _div(r, B) * G + hi, rows],
                    kv_buf.at[slot, a, i, rows], kv_sem(a, slot)))
        return copies

    def wq_copies(half, first, count):
        copies = []
        for i in range(count):
            rows = _rows((first + i) * WQ_ROWS, WQ_ROWS, WQ_ROWS)
            copies.append(pltpu.make_async_copy(
                wq_hbm[half // 2].at[rows, pl.ds((half % 2) * HW, HW)],
                wq_buf.at[half, rows], wq_sem(half)))
        return copies

    def wo_copies(br, n):
        r = n - br * BRANCH_STEPS

        def pair(k):
            return [pltpu.make_async_copy(
                wo_hbm[br].at[pl.ds(_div(r, B) * GROUP_TILES + (2 * k + i) * WO_TILES, WO_TILES)],
                wo_buf.at[wo_slot(n), pl.ds((2 * k + i) * WO_TILES, WO_TILES)],
                wo_sem(wo_slot(n))) for i in range(2)]

        pl.when(_mod(r, 4) == 3)(lambda: _start(pair(B + _div(_mod(r, B), 4))))
        return pair(_mod(r, B))

    def x_copies(br, j):
        return [pltpu.make_async_copy(
            x_hbm[br].at[_batch(j, _mod(j, G)), pl.ds(i, X_ROWS)],
            x_buf.at[br, j, pl.ds(i, X_ROWS)], x_sem(br)) for i in range(0, SQ, X_ROWS)]

    def out_copy(j, rows, cols):
        return pltpu.make_async_copy(
            out_buf.at[j, rows, cols], out.at[_batch(j, _mod(j, G)), rows, cols], out_sem)

    def start_unit(m, kv_br, wo_br=None, other=lambda m: [], by_batch=False):
        wo = [] if wo_br is None else wo_copies(wo_br, m + WO_AHEAD)
        other = other(m)
        extra = (other[:2], wo, other[2:], [])
        _start([c for chunk in range(CHUNKS)
                for c in extra[chunk] + kv_copies(kv_br, m, chunk, by_batch)])

    def start_any_unit(m, cases):
        if len(cases) == 1:
            return start_unit(m, *cases[0][1])
        half = len(cases) // 2
        lax.cond(m < cases[half][0],
                 lambda: start_any_unit(m, cases[:half]),
                 lambda: start_any_unit(m, cases[half:]))

    def q_proj(n):
        wq = wq_buf[_div(n, 4 * B), :, _rows(_mod(_div(n, B), 4) * GW, GW, GW)]
        q = jnp.dot(x_buf[_div(n, BRANCH_STEPS), _mod(n, B)], wq, preferred_element_type=F32)
        q = (q * Q_SCALE).astype(BF16)
        for h in range(G):
            q_buf[_mod(_div(n, G), Q_SLOTS), _mod(n, G), h] = q[:, h * DH:(h + 1) * DH]

    def out_proj(n):
        o = jnp.concatenate(
            [o_buf[_mod(_div(n, G), 2), _mod(n, G), h] for h in range(G)], axis=1)
        total = jnp.where(_mod(n, BRANCH_STEPS) >= B, acc[_mod(n, B)], 0.0)
        tiles = wo_buf[wo_slot(n)].reshape(GW // 8, D // DH, 8, DH)
        wo = jnp.concatenate(
            [tiles[:, c].reshape(GW, DH) for c in range(D // DH)], axis=1)
        total += jnp.dot(o, wo, preferred_element_type=F32)
        acc[_mod(n, B)] = total
        cols = _rows(_mod(_div(n, BRANCH_STEPS), 2) * D, D, DH)
        out_buf[_mod(n, B), :, cols] = total.astype(BF16)

    def probs(n, i, pos):
        s = lax.dot_general(q_buf[(_mod(_div(n, G), Q_SLOTS),) + pos],
                            kv_buf[_mod(n, KV_SLOTS), 0, i], NT_DIMS,
                            preferred_element_type=F32)
        p = jnp.exp2(s - jnp.max(s, axis=1, keepdims=True))
        return p.astype(BF16), 1.0 / jnp.sum(p, axis=1, keepdims=True)

    def values(n, i, pos, p, inv_sum):
        o = jnp.dot(p, kv_buf[_mod(n, KV_SLOTS), 1, i], preferred_element_type=F32)
        o_buf[(_mod(_div(n, G), 2),) + pos] = (o * inv_sum).astype(BF16)

    def wait_kv(n):
        for a in range(2):
            _wait_all(kv_buf.at[_mod(n, KV_SLOTS), a], kv_sem(a, _mod(n, KV_SLOTS)))

    def wait_wo(n):
        _wait_all(wo_buf.at[wo_slot(n)], wo_sem(wo_slot(n)))

    strips = D // WQ_ROWS // B
    _loop(0, B, lambda j: _start(x_copies(0, j) + wq_copies(0, strips * j, strips)))

    def clear(j):
        acc[j] = jnp.zeros((SQ, D), F32)
        for h in range(2):
            o_buf[1, _div(j, 2), 2 * _mod(j, 2) + h] = jnp.zeros((SQ, DH), BF16)
        wo_buf[WO_SLOTS - 1, pl.ds(j * (GROUP_TILES // B), GROUP_TILES // B)] = (
            jnp.zeros((GROUP_TILES // B, 8, DH), BF16))

    _loop(0, B, clear)

    rounds = KV_AHEAD * CHUNKS
    first_q = rounds - Q_AHEAD

    def prologue(j):
        pl.when(j < B)(lambda: _start(wo_copies(0, j)))
        _start(kv_copies(0, _div(j, CHUNKS), _mod(j, CHUNKS)))

        @pl.when(j == first_q)
        def _():
            _wait_all(x_buf.at[0], x_sem(0))
            _wait_all(wq_buf.at[0], wq_sem(0))

        pl.when(j >= first_q)(lambda: q_proj(j - first_q))

    _loop(0, rounds, prologue)

    def step(n):
        nq = n + Q_AHEAD
        pl.when(_mod(n, B) == G)(lambda: wait_wo(n))
        pl.when(_mod(nq, 4 * B) == 0)(
            lambda: _wait_all(wq_buf.at[_div(nq, 4 * B)], wq_sem(_div(nq, 4 * B))))
        pl.when(nq == BRANCH_STEPS)(lambda: _wait_all(x_buf.at[1], x_sem(1)))
        wait_kv(n)
        last_half = lambda m: wq_copies(3, 2 * (m - 51), 2)
        start_any_unit(n + KV_AHEAD, [
            (3, (0, 0, lambda m: wq_copies(1, 4 * (m - 3), 4))),
            (23, (0, 0, lambda m: wq_copies(2, 4 * (m - 23), 4))),
            (43, (0, 0, lambda m: x_copies(1, m - 43))),
            (51, (0, 0, last_half)),
            (BRANCH_STEPS - WO_AHEAD, (0, 1, last_half)),
            (BRANCH_STEPS, (1, 1, last_half)),
            (91, (1, 1)),
            (STEPS - WO_AHEAD, (1,)),
            (STEPS - G, (1, None, lambda m: [], True)),
        ])
        out_proj(n - G + STEPS)
        p = [probs(n, i, (i, _mod(n, G))) for i in range(G)]
        q_proj(nq)
        for i in range(G):
            values(n, i, (i, _mod(n, G)), *p[i])

    _loop(0, STEPS - Q_AHEAD, step)

    def late_step(n):
        wait_kv(n)
        p = [probs(n, i, (i, _mod(n, G))) for i in range(G)]
        out_proj(n - G)
        for i in range(G):
            values(n, i, (i, _mod(n, G)), *p[i])
        start_unit(n + KV_AHEAD, 1, by_batch=True)

    _loop(STEPS - Q_AHEAD, STEPS - G, late_step)

    wait_wo(STEPS - G)
    out_rows = [pl.ds(i, OUT_ROWS) for i in range(0, SQ, OUT_ROWS)]

    def last_step(n):
        j = _mod(n, G)
        wait_kv(n)
        pl.when(j == 1)(lambda: start_unit(STEPS - 1, 1, by_batch=True))
        pl.when(j == 2)(lambda: _start(
            [out_copy(i, rows, pl.ds(0, 2 * D)) for rows in out_rows for i in range(G)]
            + [out_copy(i, pl.ds(0, SQ), pl.ds(0, D)) for i in range(G, B)]))
        p = [probs(n, i, (j, i)) for i in range(2)]
        out_proj(STEPS - B + 2 * j)
        p += [probs(n, i, (j, i)) for i in range(2, G)]
        for i in range(G):
            values(n, i, (j, i), *p[i])
        out_proj(STEPS - B + 2 * j + 1)
        pl.when(j >= 2)(lambda: _start(
            [out_copy(2 * j + i, rows, pl.ds(D, D)) for rows in out_rows for i in range(2)]))

    _loop(STEPS - G, STEPS, last_step)

    _wait_all(out_buf, out_sem)


@jax.jit
def pallas_concat_heads__gqa_block_cached__mha_block_cached__near_ridge_kernel(
    A_x: jax.Array,
    A_k_cache: jax.Array,
    A_v_cache: jax.Array,
    A_wq: jax.Array,
    A_wo: jax.Array,
    B_x: jax.Array,
    B_k_cache: jax.Array,
    B_v_cache: jax.Array,
    B_wq: jax.Array,
    B_wo: jax.Array,
):
    def tiles(wo):
        wo = wo.reshape(H * DH // 8, 8, D // DH, DH).transpose(0, 2, 1, 3)
        return wo.reshape(-1, 8, DH)

    assert A_x.shape == B_x.shape == (B, SQ, D)
    assert A_wq.shape == B_wq.shape == (D, H * DH)
    assert all(a.shape == (B, H, SK, DH) for a in (A_k_cache, A_v_cache, B_k_cache, B_v_cache))
    args = (A_x, A_k_cache, A_v_cache, A_wq, tiles(A_wo),
            B_x, B_k_cache, B_v_cache, B_wq, tiles(B_wo))

    return pl.pallas_call(
        _kernel,
        out_shape=jax.ShapeDtypeStruct((B, SQ, 2 * D), BF16),
        in_specs=[pl.BlockSpec(memory_space=pl.ANY)] * len(args),
        out_specs=pl.BlockSpec(memory_space=pl.ANY),
        scratch_shapes=[
            pltpu.VMEM((KV_SLOTS, 2, G, SK, DH), BF16),
            pltpu.VMEM((4, D, HW), BF16),
            pltpu.VMEM((WO_SLOTS, GROUP_TILES, 8, DH), BF16),
            pltpu.VMEM((2, B, SQ, D), BF16),
            pltpu.VMEM((Q_SLOTS, G, G, SQ, DH), BF16),
            pltpu.VMEM((2, G, G, SQ, DH), BF16),
            pltpu.VMEM((B, SQ, D), F32),
            pltpu.VMEM((B, SQ, 2 * D), BF16),
            pltpu.SemaphoreType.DMA((2 * KV_SLOTS + WO_SLOTS + 7,)),
        ],
        compiler_params=pltpu.CompilerParams(
            vmem_limit_bytes=64 * 2**20, disable_bounds_checks=True),
    )(*(a.astype(BF16) for a in args))
```

```python
import math

import jax
import jax.numpy as jnp
from jax import lax
from jax.experimental import pallas as pl
from jax.experimental.pallas import tpu as pltpu

B, SQ, D = 8, 96, 640
H, SK, DH = 32, 512, 128

G = 4
GW = G * DH
HW = H * DH // 2
BRANCH_STEPS = (H // G) * B
STEPS = 2 * BRANCH_STEPS

KV_SLOTS = 4
WO_SLOTS = 4
Q_SLOTS = 4
KV_AHEAD = 3
WO_AHEAD = B - KV_AHEAD
Q_AHEAD = 5

KV_ROWS = 128
CHUNKS = SK // KV_ROWS
WQ_ROWS = 8
WO_TILES = 16
GROUP_TILES = (GW // 8) * (D // DH)
X_ROWS = 24
OUT_ROWS = 48

Q_SCALE = DH ** -0.5 * math.log2(math.e)
NT_DIMS = (((1,), (1,)), ((), ()))
F32, BF16 = jnp.float32, jnp.bfloat16


def _div(a, c):
    if isinstance(a, int):
        return a // c
    return lax.shift_right_logical(a, c.bit_length() - 1)


def _mod(a, c):
    return a & (c - 1)


def _rows(start, size, align):
    return pl.ds(start if isinstance(start, int) else pl.multiple_of(start, align), size)


def _loop(lo, hi, body):
    lax.fori_loop(lo, hi, lambda n, _: body(n), None)


def _start(copies):
    for j, copy in enumerate(copies):
        copy.start(priority=j % 2)


def _wait_all(buf, sem):
    pltpu.make_async_copy(buf, buf, sem).wait()


def _batch(n, i):
    return _mod(_div(n, G), 2) + 2 * i


def _kernel(ax, ak, av, awq, awo, bx, bk, bv, bwq, bwo, out,
            kv_buf, wq_buf, wo_buf, x_buf, q_buf, o_buf, acc, out_buf, sems):
    x_hbm, kv_hbm = (ax, bx), ((ak, av), (bk, bv))
    wq_hbm, wo_hbm = (awq, bwq), (awo, bwo)

    kv_sem = lambda a, slot: sems.at[a * KV_SLOTS + slot]
    wo_sem = lambda slot: sems.at[2 * KV_SLOTS + slot]
    wq_sem = lambda half: sems.at[2 * KV_SLOTS + WO_SLOTS + half]
    x_sem = lambda br: sems.at[2 * KV_SLOTS + WO_SLOTS + 4 + br]
    out_sem = sems.at[2 * KV_SLOTS + WO_SLOTS + 6]
    wo_slot = lambda n: _mod(_div(n, B), WO_SLOTS)

    def kv_copies(br, n, chunk, by_batch=False):
        r, slot = n - br * BRANCH_STEPS, _mod(n, KV_SLOTS)
        rows = _rows(chunk * KV_ROWS, KV_ROWS, KV_ROWS)
        copies = []
        for a in range(2):
            for i in range(G):
                bi, hi = (_mod(r, G), i) if by_batch else (i, _mod(r, G))
                copies.append(pltpu.make_async_copy(
                    kv_hbm[br][a].at[_batch(r, bi), _div(r, B) * G + hi, rows],
                    kv_buf.at[slot, a, i, rows], kv_sem(a, slot)))
        return copies

    def wq_copies(half, first, count):
        copies = []
        for i in range(count):
            rows = _rows((first + i) * WQ_ROWS, WQ_ROWS, WQ_ROWS)
            copies.append(pltpu.make_async_copy(
                wq_hbm[half // 2].at[rows, pl.ds((half % 2) * HW, HW)],
                wq_buf.at[half, rows], wq_sem(half)))
        return copies

    def wo_copies(br, n):
        r = n - br * BRANCH_STEPS

        def pair(k):
            return [pltpu.make_async_copy(
                wo_hbm[br].at[pl.ds(_div(r, B) * GROUP_TILES + (2 * k + i) * WO_TILES, WO_TILES)],
                wo_buf.at[wo_slot(n), pl.ds((2 * k + i) * WO_TILES, WO_TILES)],
                wo_sem(wo_slot(n))) for i in range(2)]

        pl.when(_mod(r, 4) == 3)(lambda: _start(pair(B + _div(_mod(r, B), 4))))
        return pair(_mod(r, B))

    def x_copies(br, j):
        return [pltpu.make_async_copy(
            x_hbm[br].at[_batch(j, _mod(j, G)), pl.ds(i, X_ROWS)],
            x_buf.at[br, j, pl.ds(i, X_ROWS)], x_sem(br)) for i in range(0, SQ, X_ROWS)]

    def out_copy(br, j, rows):
        return pltpu.make_async_copy(
            out_buf.at[br, j, rows],
            out.at[_batch(j, _mod(j, G)), rows, pl.ds(br * D, D)], out_sem)

    def start_unit(m, kv_br, wo_br=None, other=lambda m: [], by_batch=False):
        wo = [] if wo_br is None else wo_copies(wo_br, m + WO_AHEAD)
        other = other(m)
        extra = (other[:2], wo, other[2:], [])
        _start([c for chunk in range(CHUNKS)
                for c in extra[chunk] + kv_copies(kv_br, m, chunk, by_batch)])

    def start_any_unit(m, cases):
        if len(cases) == 1:
            return start_unit(m, *cases[0][1])
        half = len(cases) // 2
        lax.cond(m < cases[half][0],
                 lambda: start_any_unit(m, cases[:half]),
                 lambda: start_any_unit(m, cases[half:]))

    def q_proj(n):
        wq = wq_buf[_div(n, 4 * B), :, _rows(_mod(_div(n, B), 4) * GW, GW, GW)]
        q = jnp.dot(x_buf[_div(n, BRANCH_STEPS), _mod(n, B)], wq, preferred_element_type=F32)
        q = (q * Q_SCALE).astype(BF16)
        for h in range(G):
            q_buf[_mod(_div(n, G), Q_SLOTS), _mod(n, G), h] = q[:, h * DH:(h + 1) * DH]

    def out_proj(n):
        o = jnp.concatenate(
            [o_buf[_mod(_div(n, G), 2), _mod(n, G), h] for h in range(G)], axis=1)
        total = jnp.where(_mod(n, BRANCH_STEPS) >= B, acc[_mod(n, B)], 0.0)
        tiles = wo_buf[wo_slot(n)].reshape(GW // 8, D // DH, 8, DH)
        wo = jnp.concatenate(
            [tiles[:, c].reshape(GW, DH) for c in range(D // DH)], axis=1)
        total += jnp.dot(o, wo, preferred_element_type=F32)
        acc[_mod(n, B)] = total
        out_buf[_mod(_div(n, BRANCH_STEPS), 2), _mod(n, B)] = total.astype(BF16)

    def probs(n, i, pos):
        s = lax.dot_general(q_buf[(_mod(_div(n, G), Q_SLOTS),) + pos],
                            kv_buf[_mod(n, KV_SLOTS), 0, i], NT_DIMS,
                            preferred_element_type=F32)
        p = jnp.exp2(s - jnp.max(s, axis=1, keepdims=True))
        return p.astype(BF16), 1.0 / jnp.sum(p, axis=1, keepdims=True)

    def values(n, i, pos, p, inv_sum):
        o = jnp.dot(p, kv_buf[_mod(n, KV_SLOTS), 1, i], preferred_element_type=F32)
        o_buf[(_mod(_div(n, G), 2),) + pos] = (o * inv_sum).astype(BF16)

    def wait_kv(n):
        for a in range(2):
            _wait_all(kv_buf.at[_mod(n, KV_SLOTS), a], kv_sem(a, _mod(n, KV_SLOTS)))

    def wait_wo(n):
        _wait_all(wo_buf.at[wo_slot(n)], wo_sem(wo_slot(n)))

    strips = D // WQ_ROWS // B
    _loop(0, B, lambda j: _start(x_copies(0, j) + wq_copies(0, strips * j, strips)))

    def clear(j):
        acc[j] = jnp.zeros((SQ, D), F32)
        for h in range(2):
            o_buf[1, _div(j, 2), 2 * _mod(j, 2) + h] = jnp.zeros((SQ, DH), BF16)
        wo_buf[WO_SLOTS - 1, pl.ds(j * (GROUP_TILES // B), GROUP_TILES // B)] = (
            jnp.zeros((GROUP_TILES // B, 8, DH), BF16))

    _loop(0, B, clear)

    rounds = KV_AHEAD * CHUNKS
    first_q = rounds - Q_AHEAD

    def prologue(j):
        pl.when(j < B)(lambda: _start(wo_copies(0, j)))
        _start(kv_copies(0, _div(j, CHUNKS), _mod(j, CHUNKS)))

        @pl.when(j == first_q)
        def _():
            _wait_all(x_buf.at[0], x_sem(0))
            _wait_all(wq_buf.at[0], wq_sem(0))

        pl.when(j >= first_q)(lambda: q_proj(j - first_q))

    _loop(0, rounds, prologue)

    def step(n):
        nq = n + Q_AHEAD
        pl.when(_mod(n, B) == G)(lambda: wait_wo(n))
        pl.when(_mod(nq, 4 * B) == 0)(
            lambda: _wait_all(wq_buf.at[_div(nq, 4 * B)], wq_sem(_div(nq, 4 * B))))
        pl.when(nq == BRANCH_STEPS)(lambda: _wait_all(x_buf.at[1], x_sem(1)))
        wait_kv(n)
        last_half = lambda m: wq_copies(3, 2 * (m - 51), 2)
        start_any_unit(n + KV_AHEAD, [
            (3, (0, 0, lambda m: wq_copies(1, 4 * (m - 3), 4))),
            (23, (0, 0, lambda m: wq_copies(2, 4 * (m - 23), 4))),
            (43, (0, 0, lambda m: x_copies(1, m - 43))),
            (51, (0, 0, last_half)),
            (BRANCH_STEPS - WO_AHEAD, (0, 1, last_half)),
            (BRANCH_STEPS, (1, 1, last_half)),
            (91, (1, 1)),
            (STEPS - WO_AHEAD, (1,)),
            (STEPS - G, (1, None, lambda m: [], True)),
        ])
        out_proj(n - G + STEPS)
        p = [probs(n, i, (i, _mod(n, G))) for i in range(G)]
        q_proj(nq)
        for i in range(G):
            values(n, i, (i, _mod(n, G)), *p[i])

    _loop(0, STEPS - Q_AHEAD, step)

    def late_step(n):
        wait_kv(n)
        p = [probs(n, i, (i, _mod(n, G))) for i in range(G)]
        out_proj(n - G)
        for i in range(G):
            values(n, i, (i, _mod(n, G)), *p[i])
        start_unit(n + KV_AHEAD, 1, by_batch=True)

    _loop(STEPS - Q_AHEAD, STEPS - G, late_step)

    wait_wo(STEPS - G)
    out_rows = [pl.ds(i, OUT_ROWS) for i in range(0, SQ, OUT_ROWS)]

    def last_step(n):
        j = _mod(n, G)
        wait_kv(n)
        pl.when(j == 1)(lambda: start_unit(STEPS - 1, 1, by_batch=True))
        pl.when(j == 2)(lambda: _start(
            [out_copy(br, i, pl.ds(0, SQ)) for br, done in ((0, B), (1, G)) for i in range(done)]))
        p = [probs(n, i, (j, i)) for i in range(2)]
        out_proj(STEPS - B + 2 * j)
        p += [probs(n, i, (j, i)) for i in range(2, G)]
        for i in range(G):
            values(n, i, (j, i), *p[i])
        out_proj(STEPS - B + 2 * j + 1)
        pl.when(j >= 2)(lambda: _start(
            [out_copy(1, 2 * j + i, rows) for rows in out_rows for i in range(2)]))

    _loop(STEPS - G, STEPS, last_step)

    _wait_all(out, out_sem)


@jax.jit
def pallas_concat_heads__gqa_block_cached__mha_block_cached__near_ridge_kernel(
    A_x: jax.Array,
    A_k_cache: jax.Array,
    A_v_cache: jax.Array,
    A_wq: jax.Array,
    A_wo: jax.Array,
    B_x: jax.Array,
    B_k_cache: jax.Array,
    B_v_cache: jax.Array,
    B_wq: jax.Array,
    B_wo: jax.Array,
):
    def tiles(wo):
        wo = wo.reshape(H * DH // 8, 8, D // DH, DH).transpose(0, 2, 1, 3)
        return wo.reshape(-1, 8, DH)

    assert A_x.shape == B_x.shape == (B, SQ, D)
    assert A_wq.shape == B_wq.shape == (D, H * DH)
    assert all(a.shape == (B, H, SK, DH) for a in (A_k_cache, A_v_cache, B_k_cache, B_v_cache))
    args = (A_x, A_k_cache, A_v_cache, A_wq, tiles(A_wo),
            B_x, B_k_cache, B_v_cache, B_wq, tiles(B_wo))

    return pl.pallas_call(
        _kernel,
        out_shape=jax.ShapeDtypeStruct((B, SQ, 2 * D), BF16),
        in_specs=[pl.BlockSpec(memory_space=pl.ANY)] * len(args),
        out_specs=pl.BlockSpec(memory_space=pl.ANY),
        scratch_shapes=[
            pltpu.VMEM((KV_SLOTS, 2, G, SK, DH), BF16),
            pltpu.VMEM((4, D, HW), BF16),
            pltpu.VMEM((WO_SLOTS, GROUP_TILES, 8, DH), BF16),
            pltpu.VMEM((2, B, SQ, D), BF16),
            pltpu.VMEM((Q_SLOTS, G, G, SQ, DH), BF16),
            pltpu.VMEM((2, G, G, SQ, DH), BF16),
            pltpu.VMEM((B, SQ, D), F32),
            pltpu.VMEM((2, B, SQ, D), BF16),
            pltpu.SemaphoreType.DMA((2 * KV_SLOTS + WO_SLOTS + 7,)),
        ],
        compiler_params=pltpu.CompilerParams(
            vmem_limit_bytes=64 * 2**20, disable_bounds_checks=True),
    )(*(a.astype(BF16) for a in args))
```
